```python
import os as _os
_os.environ.setdefault("JAX_PLATFORMS", "cpu")
import jax
import jax.numpy as jnp

def _softmax(x, axis=-1):
    return jax.nn.softmax(x, axis=axis)
def _gelu(x):
    return jax.nn.gelu(x, approximate=True)
def _silu(x):
    return jax.nn.silu(x)
def _sigmoid(x):
    return jax.nn.sigmoid(x)
def _layernorm(x, axis=-1, eps=1e-5):
    m = jnp.mean(x, axis=axis, keepdims=True)
    v = jnp.var(x, axis=axis, keepdims=True)
    return (x - m) / jnp.sqrt(v + eps)
def _scatter_add(tgt, idx, src, axis=0):
    return tgt.at[idx].add(src)
def _segment_sum(src, seg, n):
    return jax.ops.segment_sum(src, seg, n)
class _Rng:
    def __init__(self, key):
        self._k = key
    def _next(self):
        self._k, sub = jax.random.split(self._k)
        return sub
    def normal(self, shape):
        return jax.random.normal(self._next(), shape, dtype=jnp.bfloat16)
    def randint(self, lo, hi, shape):
        return jax.random.randint(self._next(), shape, lo, hi, dtype=jnp.int32)
    def uniform(self, shape, lo=0.0, hi=1.0):
        return jax.random.uniform(self._next(), shape, jnp.bfloat16, lo, hi)
    def permutation(self, n):
        return jax.random.permutation(self._next(), n)


kernel_name = 'concat_heads__sliding_block_cached__sliding_block_cached__decode'

def setup_inputs():
    _rng = _Rng(jax.random.key(int.from_bytes(__import__("os").urandom(4), "little")))
    _w = (lambda a: (lambda t: t.astype(jnp.bfloat16) if jnp.issubdtype(t.dtype, jnp.floating) else t)(jnp.asarray(a)))
    def _A_setup():
        B, Sq, D = 2, 1, 640
        Hq, Hkv, Sk, Dh = 32, 32, 4096, 128
        assert Hq % Hkv == 0, (Hq, Hkv)
        return {
            "x": _w((lambda *s: _rng.normal(s) * 0.8)(B, Sq, D)),
            "k_cache": _w((lambda *s: _rng.normal(s) * 0.8)(B, Hkv, Sk, Dh)),
            "v_cache": _w((lambda *s: _rng.normal(s) * 0.05)(B, Hkv, Sk, Dh)),
            "wq": _w((lambda *s: _rng.normal(s) * 0.8)(D, Hq * Dh) * (D ** -0.5)),
            "wo": _w((lambda *s: _rng.normal(s) * 0.05)(Hq * Dh, D) * ((Hq * Dh) ** -0.5)),
        }
    _A_in = _A_setup()

    def _B_setup():
        B, Sq, D = 2, 1, 640
        Hq, Hkv, Sk, Dh = 32, 32, 4096, 128
        assert Hq % Hkv == 0, (Hq, Hkv)
        return {
            "x": _w((lambda *s: _rng.normal(s) * 0.8)(B, Sq, D)),
            "k_cache": _w((lambda *s: _rng.normal(s) * 0.8)(B, Hkv, Sk, Dh)),
            "v_cache": _w((lambda *s: _rng.normal(s) * 0.05)(B, Hkv, Sk, Dh)),
            "wq": _w((lambda *s: _rng.normal(s) * 0.8)(D, Hq * Dh) * (D ** -0.5)),
            "wo": _w((lambda *s: _rng.normal(s) * 0.05)(Hq * Dh, D) * ((Hq * Dh) ** -0.5)),
        }
    _B_in = _B_setup()

    return {
        "A_x": _A_in["x"],
        "A_k_cache": _A_in["k_cache"],
        "A_v_cache": _A_in["v_cache"],
        "A_wq": _A_in["wq"],
        "A_wo": _A_in["wo"],
        "B_x": _B_in["x"],
        "B_k_cache": _B_in["k_cache"],
        "B_v_cache": _B_in["v_cache"],
        "B_wq": _B_in["wq"],
        "B_wo": _B_in["wo"],
    }

def reference(A_x, A_k_cache, A_v_cache, A_wq, A_wo, B_x, B_k_cache, B_v_cache, B_wq, B_wo):
    def _A_ref(x, k_cache, v_cache, wq, wo):
        B, Sq, D = x.shape
        Hq, Dh = 32, 128
        Hkv, Sk = k_cache.shape[1], k_cache.shape[2]
        W = min(4096, max(256, Sk // 4))
        rep = Hq // Hkv
        q = (lambda x, *d: x.transpose(*d))((x @ wq).reshape(B, Sq, Hq, Dh), 0, 2, 1, 3)
        k = jnp.repeat(k_cache[:, :, Sk - W:, :], rep, axis=1)
        v = jnp.repeat(v_cache[:, :, Sk - W:, :], rep, axis=1)
        scores = jnp.einsum("bhqd,bhkd->bhqk", q, k) * (Dh ** -0.5)
        p = _softmax(scores, axis=-1)
        o = jnp.einsum("bhqk,bhkd->bhqd", p, v)
        return (lambda x, *d: x.transpose(*d))(o, 0, 2, 1, 3).reshape(B, Sq, Hq * Dh) @ wo

    def _B_ref(x, k_cache, v_cache, wq, wo):
        B, Sq, D = x.shape
        Hq, Dh = 32, 128
        Hkv, Sk = k_cache.shape[1], k_cache.shape[2]
        W = min(4096, max(256, Sk // 4))
        rep = Hq // Hkv
        q = (lambda x, *d: x.transpose(*d))((x @ wq).reshape(B, Sq, Hq, Dh), 0, 2, 1, 3)
        k = jnp.repeat(k_cache[:, :, Sk - W:, :], rep, axis=1)
        v = jnp.repeat(v_cache[:, :, Sk - W:, :], rep, axis=1)
        scores = jnp.einsum("bhqd,bhkd->bhqk", q, k) * (Dh ** -0.5)
        p = _softmax(scores, axis=-1)
        o = jnp.einsum("bhqk,bhkd->bhqd", p, v)
        return (lambda x, *d: x.transpose(*d))(o, 0, 2, 1, 3).reshape(B, Sq, Hq * Dh) @ wo

    a = _A_ref(A_x, A_k_cache, A_v_cache, A_wq, A_wo)
    b = _B_ref(B_x, B_k_cache, B_v_cache, B_wq, B_wo)
    return jnp.concatenate([a, b], axis=-1)
```

```python
import jax
import jax.numpy as jnp
from jax import lax
import jax.experimental.pallas as pl
import jax.experimental.pallas.tpu as pltpu

H, DH, D, SK, NB = 32, 128, 640, 4096, 2
W = min(4096, max(256, SK // 4))

KV_ROWS = 32
WO_ROWS = 16
WQ_COLS = 512
WQ_PH = 5


def _kernel(ax, ak, av, awq, awo, bx, bk, bv, bwq, bwo, o_ref,
            xbuf, wqbuf, qbuf, kbuf, vbuf, wobuf, xsem, wqsem, ksem, vsem, osem):
    cnt = [0]

    def go(copy):
        copy.start(priority=cnt[0] % 2)
        cnt[0] += 1

    def issue_kv(a_ref, b_ref, buf, sem, slot, h):
        for r in range(W // KV_ROWS):
            for s, ref in enumerate((a_ref, b_ref)):
                for b in range(NB):
                    go(pltpu.make_async_copy(
                        ref.at[b, h, pl.ds(SK - W + r * KV_ROWS, KV_ROWS), :],
                        buf.at[slot, 2 * s + b, pl.ds(r * KV_ROWS, KV_ROWS), :],
                        sem.at[slot]))

    def issue_wo(slot, h):
        for r in range(DH // WO_ROWS):
            for s, ref in enumerate((awo, bwo)):
                go(pltpu.make_async_copy(
                    ref.at[pl.ds(h * DH + r * WO_ROWS, WO_ROWS), :],
                    wobuf.at[slot, s, pl.ds(r * WO_ROWS, WO_ROWS), :],
                    osem.at[slot]))

    def wait_all(buf, sem, slot):
        pltpu.make_async_copy(buf.at[slot], buf.at[slot], sem.at[slot]).wait()

    def issue_wq(ph):
        s, rb = divmod(ph, WQ_PH)
        ref = (awq, bwq)[s]
        for r in range(128 // 16):
            for c in range(H * DH // WQ_COLS):
                r0 = rb * 128 + r * 16
                go(pltpu.make_async_copy(
                    ref.at[pl.ds(r0, 16), pl.ds(c * WQ_COLS, WQ_COLS)],
                    wqbuf.at[s, pl.ds(r0, 16), pl.ds(c * WQ_COLS, WQ_COLS)],
                    wqsem.at[ph]))

    def wait_wq(ph):
        s, rb = divmod(ph, WQ_PH)
        dst = wqbuf.at[s, pl.ds(rb * 128, 128), :]
        pltpu.make_async_copy(dst, dst, wqsem.at[ph]).wait()

    def compute_q(s):
        x = xbuf[s, :, 0, :]
        q = jnp.dot(x, wqbuf[s], preferred_element_type=jnp.float32).astype(jnp.bfloat16)
        for h in range(H):
            qbuf[h, pl.ds(2 * s, 2), :] = q[:, h * DH:(h + 1) * DH]

    cx = [pltpu.make_async_copy(ax, xbuf.at[0], xsem.at[0]),
          pltpu.make_async_copy(bx, xbuf.at[1], xsem.at[1])]
    issue_wq(0)
    cx[0].start()
    cx[1].start()
    issue_wq(1)
    n_ph = 2 * WQ_PH
    for ph in range(n_ph):
        wait_wq(ph)
        nxt = ph + 2
        if nxt < n_ph:
            issue_wq(nxt)
        elif nxt == n_ph:
            issue_kv(ak, bk, kbuf, ksem, 0, 0)
        else:
            issue_kv(av, bv, vbuf, vsem, 0, 0)
            issue_wo(0, 0)
        if ph % WQ_PH == WQ_PH - 1:
            cx[ph // WQ_PH].wait()
            compute_q(ph // WQ_PH)

    row_w = lax.broadcasted_iota(jnp.int32, (4, W), 0)
    row_h = lax.broadcasted_iota(jnp.int32, (4, DH), 0)
    row_d = lax.broadcasted_iota(jnp.int32, (4, D), 0)
    scale = DH ** -0.5
    nt_dims = (((1,), (1,)), ((), ()))

    def pick(row, xs):
        return jnp.where(row < 2, jnp.where(row == 0, xs[0], xs[1]),
                         jnp.where(row == 2, xs[2], xs[3]))

    def unit(h, slot, acc, last=False):
        q4 = qbuf[h]
        wait_all(kbuf, ksem, slot)
        if not last:
            issue_kv(ak, bk, kbuf, ksem, 1 - slot, h + 1)
        ss = [lax.dot_general(q4, kbuf[slot, i], nt_dims, preferred_element_type=jnp.float32)
              for i in range(4)]
        s = pick(row_w, ss) * scale
        m = jnp.max(s, axis=-1, keepdims=True)
        p = jnp.exp(s - m)
        l = jnp.sum(p, axis=-1, keepdims=True)
        pb = p.astype(jnp.bfloat16)
        wait_all(vbuf, vsem, slot)
        if not last:
            issue_kv(av, bv, vbuf, vsem, 1 - slot, h + 1)
            issue_wo(1 - slot, h + 1)
        os_ = [jnp.dot(pb, vbuf[slot, i], preferred_element_type=jnp.float32) for i in range(4)]
        ob = (pick(row_h, os_) / l).astype(jnp.bfloat16)
        wait_all(wobuf, osem, slot)
        ra = jnp.dot(ob, wobuf[slot, 0], preferred_element_type=jnp.float32)
        rb = jnp.dot(ob, wobuf[slot, 1], preferred_element_type=jnp.float32)
        return acc + jnp.where(row_d < 2, ra, rb)

    def body(i, acc):
        acc = unit(2 * i, 0, acc)
        return unit(2 * i + 1, 1, acc)

    acc = lax.fori_loop(0, H // 2 - 1, body, jnp.zeros((4, D), jnp.float32))
    acc = unit(H - 2, 0, acc)
    acc = unit(H - 1, 1, acc, last=True)
    res = acc.astype(o_ref.dtype)
    o_ref[:, 0, 0:D] = res[0:2]
    o_ref[:, 0, D:2 * D] = res[2:4]


@jax.jit
def pallas_concat_heads__sliding_block_cached__sliding_block_cached__decode_kernel(
    A_x: jax.Array,
    A_k_cache: jax.Array,
    A_v_cache: jax.Array,
    A_wq: jax.Array,
    A_wo: jax.Array,
    B_x: jax.Array,
    B_k_cache: jax.Array,
    B_v_cache: jax.Array,
    B_wq: jax.Array,
    B_wo: jax.Array,
):
    return pl.pallas_call(
        _kernel,
        out_shape=jax.ShapeDtypeStruct((NB, 1, 2 * D), A_x.dtype),
        in_specs=[pl.BlockSpec(memory_space=pl.ANY)] * 10,
        out_specs=pl.BlockSpec(memory_space=pltpu.VMEM),
        scratch_shapes=[
            pltpu.VMEM((2, NB, 1, D), jnp.bfloat16),
            pltpu.VMEM((2, D, H * DH), jnp.bfloat16),
            pltpu.VMEM((H, 4, DH), jnp.bfloat16),
            pltpu.VMEM((2, 4, W, DH), jnp.bfloat16),
            pltpu.VMEM((2, 4, W, DH), jnp.bfloat16),
            pltpu.VMEM((2, 2, DH, D), jnp.bfloat16),
            pltpu.SemaphoreType.DMA((2,)),
            pltpu.SemaphoreType.DMA((2 * WQ_PH,)),
            pltpu.SemaphoreType.DMA((2,)),
            pltpu.SemaphoreType.DMA((2,)),
            pltpu.SemaphoreType.DMA((2,)),
        ],
        compiler_params=pltpu.CompilerParams(vmem_limit_bytes=64 * 1024 * 1024),
    )(A_x, A_k_cache, A_v_cache, A_wq, A_wo, B_x, B_k_cache, B_v_cache, B_wq, B_wo)
```

```python
import jax
import jax.numpy as jnp
from jax import lax
import jax.experimental.pallas as pl
import jax.experimental.pallas.tpu as pltpu

H, DH, D, SK, NB = 32, 128, 640, 4096, 2
W = min(4096, max(256, SK // 4))

KV_ROWS = 64
WO_ROWS = 16
WQ_ROWS = 8
WQ_COLS = 1024
WQ_PROWS = 320
HALVES = ((0, 0), (0, 1), (1, 0), (1, 1))


def _kernel(ax, ak, av, awq, awo, bx, bk, bv, bwq, bwo, o_ref,
            xbuf, wqbuf, kbuf, vbuf, wobuf, ksem, vsem, osem):
    cnt = [0]

    def start_all(copies):
        for c in copies:
            c.start(priority=cnt[0] % 2)
            cnt[0] += 1

    def issue_kv(a_ref, b_ref, buf, sem, slot, h):
        copies = []
        for r in range(W // KV_ROWS):
            for it in range(4):
                s, b = divmod(it, 2)
                copies.append(pltpu.make_async_copy(
                    (a_ref, b_ref)[s].at[b, h, pl.ds(SK - W + r * KV_ROWS, KV_ROWS), :],
                    buf.at[slot, it, pl.ds(r * KV_ROWS, KV_ROWS), :],
                    sem.at[slot]))
        start_all(copies)

    def issue_k(slot, h):
        issue_kv(ak, bk, kbuf, ksem, slot, h)

    def issue_v(slot, h):
        issue_kv(av, bv, vbuf, vsem, slot, h)

    def issue_wo(slot, h):
        n = DH // WO_ROWS // 2
        copies = []
        for r0 in range(n):
            for s, half in HALVES:
                r = r0 + half * n
                copies.append(pltpu.make_async_copy(
                    (awo, bwo)[s].at[pl.ds(h * DH + r * WO_ROWS, WO_ROWS), :],
                    wobuf.at[slot, s, pl.ds(r * WO_ROWS, WO_ROWS), :],
                    osem.at[slot]))
        start_all(copies)

    def wait_all(buf, sem, slot):
        pltpu.make_async_copy(buf.at[slot], buf.at[slot], sem.at[slot]).wait()

    def issue_wq(ph):
        n = WQ_PROWS // WQ_ROWS // 2
        copies = []
        for r0 in range(n):
            for c in range(H * DH // WQ_COLS):
                for s, half in HALVES:
                    rows = pl.ds(ph * WQ_PROWS + (r0 + half * n) * WQ_ROWS, WQ_ROWS)
                    cols = pl.ds(c * WQ_COLS, WQ_COLS)
                    copies.append(pltpu.make_async_copy(
                        (awq, bwq)[s].at[rows, cols], wqbuf.at[s, rows, cols], ksem.at[ph]))
        start_all(copies)

    def wait_wq(ph):
        dst = wqbuf.at[:, pl.ds(ph * WQ_PROWS, WQ_PROWS), :]
        pltpu.make_async_copy(dst, dst, ksem.at[ph]).wait()

    cx = [pltpu.make_async_copy(ax, xbuf.at[0], vsem.at[1]),
          pltpu.make_async_copy(bx, xbuf.at[1], osem.at[1])]
    issue_wq(0)
    cx[0].start()
    cx[1].start()
    issue_wq(1)
    wait_wq(0)
    issue_k(0, 0)
    wait_wq(1)
    issue_v(0, 0)
    issue_wo(0, 0)
    cx[0].wait()
    cx[1].wait()

    row_w = lax.broadcasted_iota(jnp.int32, (4, W), 0)
    row_h = lax.broadcasted_iota(jnp.int32, (4, DH), 0)
    row_d = lax.broadcasted_iota(jnp.int32, (4, D), 0)
    scale = DH ** -0.5
    nt_dims = (((1,), (1,)), ((), ()))

    def pick(row, xs):
        return jnp.where(row < 2, jnp.where(row == 0, xs[0], xs[1]),
                         jnp.where(row == 2, xs[2], xs[3]))

    def get_q(h):
        cols = pl.ds(pl.multiple_of(h * DH, DH), DH)
        qa = jnp.dot(xbuf[0], wqbuf[0, :, cols], preferred_element_type=jnp.float32)
        qb = jnp.dot(xbuf[1], wqbuf[1, :, cols], preferred_element_type=jnp.float32)
        return jnp.concatenate([qa, qb], axis=0).astype(jnp.bfloat16)

    def attend(q4, slot, after_k, after_v, next_head):
        wait_all(kbuf, ksem, slot)
        after_k()
        ss = [lax.dot_general(q4, kbuf[slot, i], nt_dims, preferred_element_type=jnp.float32)
              for i in range(4)]
        s = pick(row_w, ss) * scale
        m = jnp.max(s, axis=-1, keepdims=True)
        p = jnp.exp(s - m)
        l = jnp.sum(p, axis=-1, keepdims=True)
        pb = p.astype(jnp.bfloat16)
        qn = q4 if next_head is None else get_q(next_head)
        wait_all(vbuf, vsem, slot)
        after_v()
        os_ = [jnp.dot(pb, vbuf[slot, i], preferred_element_type=jnp.float32) for i in range(4)]
        return (pick(row_h, os_) / l).astype(jnp.bfloat16), qn

    def out_proj(ob, slot, acc):
        wait_all(wobuf, osem, slot)
        ra = jnp.dot(ob, wobuf[slot, 0], preferred_element_type=jnp.float32)
        rb = jnp.dot(ob, wobuf[slot, 1], preferred_element_type=jnp.float32)
        return acc + jnp.where(row_d < 2, ra, rb)

    def nothing():
        pass

    def body(i, carry):
        acc, q4 = carry
        h = 2 * i

        def after_v0():
            issue_v(1, h + 1)
            issue_wo(1, h + 1)

        ob, q4 = attend(q4, 0, lambda: issue_k(1, h + 1), after_v0, h + 1)
        acc = out_proj(ob, 0, acc)

        def after_v1():
            issue_v(0, h + 2)

            @pl.when(i < H // 2 - 2)
            def _():
                issue_wo(0, h + 2)

        ob, q4 = attend(q4, 1, lambda: issue_k(0, h + 2), after_v1, h + 2)
        return out_proj(ob, 1, acc), q4

    acc, q4 = lax.fori_loop(0, H // 2 - 1, body, (jnp.zeros((4, D), jnp.float32), get_q(0)))

    def after_v_last():
        issue_v(1, H - 1)
        issue_wo(0, H - 2)
        issue_wo(1, H - 1)

    ob0, q4 = attend(q4, 0, lambda: issue_k(1, H - 1), after_v_last, H - 1)
    ob1, _ = attend(q4, 1, nothing, nothing, None)
    acc = out_proj(ob0, 0, acc)
    acc = out_proj(ob1, 1, acc)
    res = acc.astype(o_ref.dtype)
    o_ref[:, 0:D] = res[0:2]
    o_ref[:, D:2 * D] = res[2:4]


@jax.jit
def pallas_concat_heads__sliding_block_cached__sliding_block_cached__decode_kernel(
    A_x: jax.Array,
    A_k_cache: jax.Array,
    A_v_cache: jax.Array,
    A_wq: jax.Array,
    A_wo: jax.Array,
    B_x: jax.Array,
    B_k_cache: jax.Array,
    B_v_cache: jax.Array,
    B_wq: jax.Array,
    B_wo: jax.Array,
):
    out = pl.pallas_call(
        _kernel,
        out_shape=jax.ShapeDtypeStruct((NB, 2 * D), A_x.dtype),
        in_specs=[pl.BlockSpec(memory_space=pl.ANY)] * 10,
        out_specs=pl.BlockSpec(memory_space=pltpu.VMEM),
        scratch_shapes=[
            pltpu.VMEM((2, NB, D), jnp.bfloat16),
            pltpu.VMEM((2, D, H * DH), jnp.bfloat16),
            pltpu.VMEM((2, 4, W, DH), jnp.bfloat16),
            pltpu.VMEM((2, 4, W, DH), jnp.bfloat16),
            pltpu.VMEM((2, 2, DH, D), jnp.bfloat16),
            pltpu.SemaphoreType.DMA((2,)),
            pltpu.SemaphoreType.DMA((2,)),
            pltpu.SemaphoreType.DMA((2,)),
        ],
        compiler_params=pltpu.CompilerParams(vmem_limit_bytes=64 * 1024 * 1024),
    )(A_x.reshape(NB, D), A_k_cache, A_v_cache, A_wq, A_wo,
      B_x.reshape(NB, D), B_k_cache, B_v_cache, B_wq, B_wo)
    return out.reshape(NB, 1, 2 * D)
```
